```python
import os as _os
_os.environ.setdefault("JAX_PLATFORMS", "cpu")
import jax
import jax.numpy as jnp

def _softmax(x, axis=-1):
    return jax.nn.softmax(x, axis=axis)
def _gelu(x):
    return jax.nn.gelu(x, approximate=True)
def _silu(x):
    return jax.nn.silu(x)
def _sigmoid(x):
    return jax.nn.sigmoid(x)
def _layernorm(x, axis=-1, eps=1e-5):
    m = jnp.mean(x, axis=axis, keepdims=True)
    v = jnp.var(x, axis=axis, keepdims=True)
    return (x - m) / jnp.sqrt(v + eps)
def _scatter_add(tgt, idx, src, axis=0):
    return tgt.at[idx].add(src)
def _segment_sum(src, seg, n):
    return jax.ops.segment_sum(src, seg, n)
class _Rng:
    def __init__(self, key):
        self._k = key
    def _next(self):
        self._k, sub = jax.random.split(self._k)
        return sub
    def normal(self, shape):
        return jax.random.normal(self._next(), shape, dtype=jnp.bfloat16)
    def randint(self, lo, hi, shape):
        return jax.random.randint(self._next(), shape, lo, hi, dtype=jnp.int32)
    def uniform(self, shape, lo=0.0, hi=1.0):
        return jax.random.uniform(self._next(), shape, jnp.bfloat16, lo, hi)
    def permutation(self, n):
        return jax.random.permutation(self._next(), n)


kernel_name = 'interleave_layers__sliding_block_cached__mixer_channel_mlp__decode'

def setup_inputs():
    _rng = _Rng(jax.random.key(int.from_bytes(__import__("os").urandom(4), "little")))
    _w = (lambda a: (lambda t: t.astype(jnp.bfloat16) if jnp.issubdtype(t.dtype, jnp.floating) else t)(jnp.asarray(a)))
    def _A_setup():
        B, Sq, D = 8, 1, 1024
        Hq, Hkv, Sk, Dh = 32, 4, 4096, 128
        assert Hq % Hkv == 0, (Hq, Hkv)
        return {
            "x": _w((lambda *s: _rng.normal(s) * 0.05)(B, Sq, D)),
            "k_cache": _w((lambda *s: _rng.normal(s) * 1.6)(B, Hkv, Sk, Dh)),
            "v_cache": _w((lambda *s: _rng.normal(s) * 0.8)(B, Hkv, Sk, Dh)),
            "wq": _w((lambda *s: _rng.normal(s) * 1.6)(D, Hq * Dh) * (D ** -0.5)),
            "wo": _w((lambda *s: _rng.normal(s) * 0.8)(Hq * Dh, D) * ((Hq * Dh) ** -0.5)),
        }
    _A_in = _A_setup()

    def _B_setup():
        B, S, D, F = 8, 1, 1024, 3584
        return {
            "x": _w((lambda *s: _rng.normal(s) * 0.05)(B, S, D)),
            "w1": _w((lambda *s: _rng.normal(s) * 0.4)(D, F) * (D ** -0.5)),
            "b1": _w((lambda *s: _rng.normal(s) * 0.4)(F)),
            "w2": _w((lambda *s: _rng.normal(s) * 0.4)(F, D) * (F ** -0.5)),
            "b2": _w((lambda *s: _rng.normal(s) * 0.1)(D)),
        }
    _B_in = _B_setup()

    return {
        "A_x": _A_in["x"],
        "A_k_cache": _A_in["k_cache"],
        "A_v_cache": _A_in["v_cache"],
        "A_wq": _A_in["wq"],
        "A_wo": _A_in["wo"],
        "B_x": _B_in["x"],
        "B_w1": _B_in["w1"],
        "B_b1": _B_in["b1"],
        "B_w2": _B_in["w2"],
        "B_b2": _B_in["b2"],
    }

def reference(A_x, A_k_cache, A_v_cache, A_wq, A_wo, B_x, B_w1, B_b1, B_w2, B_b2):
    def _A_ref(x, k_cache, v_cache, wq, wo):
        B, Sq, D = x.shape
        Hq, Dh = 32, 128
        Hkv, Sk = k_cache.shape[1], k_cache.shape[2]
        W = min(4096, max(256, Sk // 4))
        rep = Hq // Hkv
        q = (lambda x, *d: x.transpose(*d))((x @ wq).reshape(B, Sq, Hq, Dh), 0, 2, 1, 3)
        k = jnp.repeat(k_cache[:, :, Sk - W:, :], rep, axis=1)
        v = jnp.repeat(v_cache[:, :, Sk - W:, :], rep, axis=1)
        scores = jnp.einsum("bhqd,bhkd->bhqk", q, k) * (Dh ** -0.5)
        p = _softmax(scores, axis=-1)
        o = jnp.einsum("bhqk,bhkd->bhqd", p, v)
        return (lambda x, *d: x.transpose(*d))(o, 0, 2, 1, 3).reshape(B, Sq, Hq * Dh) @ wo

    def _B_ref(x, w1, b1, w2, b2):
        y = _layernorm(x, axis=-1)
        h = _gelu(jnp.einsum("bsd,df->bsf", y, w1) + b1)
        return jnp.einsum("bsf,fd->bsd", h, w2) + b2

    x = A_x
    x = x + _A_ref(_layernorm(x, axis=-1), A_k_cache, A_v_cache, A_wq, A_wo)
    x = x + _B_ref(_layernorm(x, axis=-1), B_w1, B_b1, B_w2, B_b2)
    x = x + _A_ref(_layernorm(x, axis=-1), A_k_cache, A_v_cache, A_wq, A_wo)
    x = x + _B_ref(_layernorm(x, axis=-1), B_w1, B_b1, B_w2, B_b2)
    return x
```

```python
import functools

import jax
import jax.numpy as jnp
import jax.experimental.pallas as pl
import jax.experimental.pallas.tpu as pltpu

F32 = jnp.float32
BF16 = jnp.bfloat16
U32 = jnp.uint32
EPS = 1e-5
LANE = 128


def _stats(x):
    m = jnp.mean(x, axis=-1, keepdims=True)
    d = x - m
    v = jnp.mean(d * d, axis=-1, keepdims=True)
    return m, v, d


def _ln(x):
    _, v, d = _stats(x)
    return d * jax.lax.rsqrt(v + EPS)


def _hilo(x):
    hi = x.astype(BF16).astype(F32)
    return jnp.concatenate([hi, x - hi], axis=0).astype(BF16)


def _with_ones(x):
    r = jax.lax.broadcasted_iota(jnp.int32, x.shape, 0)
    ones = jnp.where(r == 0, 1.0, 0.0).astype(F32)
    return jnp.concatenate([x, ones], axis=0).astype(BF16)


def _dot(a, b):
    return jnp.dot(a, b, preferred_element_type=F32)


def _dot_nt(a, b):
    return jax.lax.dot_general(a, b, (((1,), (1,)), ((), ())), preferred_element_type=F32)


class Unit:
    def __init__(self, n, piece, whole):
        self.n = n
        self.piece = piece
        self.whole = whole
        self.sem = None


def make_kernel(B, D, Hq, Hkv, Sk, Dh, F, W, cfg):
    rep = Hq // Hkv
    G = B * Hkv
    HD = Hq * Dh
    T = cfg["tail_rows"]
    R = F - T
    tail_cols = cfg["tail_cols"]
    scale = Dh ** -0.5
    NF = F // LANE
    ND = D // LANE
    L = cfg["lag"]
    UN = cfg["unroll"]
    m0, m1 = cfg["margin0"], cfg["margin1"]
    NQ = 4
    n_sems = 3 + 6 * NQ + len(tail_cols)

    def kernel(x_hbm, k_hbm, v_hbm, wq_hbm, wo_hbm, w1_hbm, b1_hbm, w2_hbm, b2_hbm,
               o_ref,
               x_v, b1_v, b2_v,
               wq_s, k_s, v_s, wo_s, w1_s, w2_s, w2t,
               wq_p, kt_p, wo_p, w1_p, w2_p,
               q_scr, o_scr, s_scr,
               sems):
        sem_ctr = [0]

        def new_sem():
            s = sems.at[sem_ctr[0]]
            sem_ctr[0] += 1
            return s

        def small(src, dst):
            c = pltpu.make_async_copy(src, dst, new_sem())
            c.start(priority=0)
            return c

        def rows_unit(hbm, stage, r0, rc, prow, ncol):
            N = hbm.shape[1]
            cw = N // ncol
            n = rc // prow * ncol

            def piece(i):
                r = r0 + (i // ncol) * prow
                if not isinstance(r, int):
                    r = pl.multiple_of(r, prow)
                if ncol == 1:
                    return hbm.at[pl.ds(r, prow)], stage.at[pl.ds(r, prow)]
                c = (i % ncol) * cw
                if not isinstance(c, int):
                    c = pl.multiple_of(c, LANE)
                return hbm.at[pl.ds(r, prow), pl.ds(c, cw)], stage.at[pl.ds(r, prow), pl.ds(c, cw)]

            return Unit(n, piece, lambda: (hbm.at[pl.ds(r0, rc)], stage.at[pl.ds(r0, rc)]))

        def kv_unit(hbm, stage, b0, nb, prow):
            per = W // prow
            n = nb * Hkv * per

            def piece(i):
                g = i // per
                r = (i % per) * prow
                if not isinstance(r, int):
                    r = pl.multiple_of(r, prow)
                b = b0 + g // Hkv
                kv = g % Hkv
                return (hbm.at[b, kv, pl.ds(Sk - W + r, prow), :], stage.at[b, kv, pl.ds(r, prow), :])

            return Unit(n, piece, lambda: (hbm.at[pl.ds(b0, nb), :, pl.ds(Sk - W, W), :],
                                           stage.at[pl.ds(b0, nb)]))

        def tail_unit(j0, nj, prow, rb0=0, nrb=None):
            rows0 = rb0 * prow
            nrows = T - rows0 if nrb is None else nrb * prow
            n = nrows // prow * nj

            def piece(i):
                r = rows0 + (i // nj) * prow
                j = j0 + i % nj
                c = j * LANE
                if not isinstance(r, int):
                    r = pl.multiple_of(r, prow)
                    c = pl.multiple_of(c, LANE)
                return (w2_hbm.at[pl.ds(R + r, prow), pl.ds(c, LANE)], w2t.at[j, pl.ds(r, prow), :])

            return Unit(n, piece, lambda: (w2t.at[pl.ds(j0, nj)], w2t.at[pl.ds(j0, nj)]))

        u_wq = [rows_unit(wq_hbm, wq_s, i * (D // NQ), D // NQ, 8, 2) for i in range(NQ)]
        u_k = [kv_unit(k_hbm, k_s, i * (B // NQ), B // NQ, 128) for i in range(NQ)]
        u_v = [kv_unit(v_hbm, v_s, i * (B // NQ), B // NQ, 128) for i in range(NQ)]
        u_wo = [rows_unit(wo_hbm, wo_s, i * (HD // NQ), HD // NQ, 16, 1) for i in range(NQ)]
        u_w1 = [rows_unit(w1_hbm, w1_s, i * (D // NQ), D // NQ, 8, 2) for i in range(NQ)]
        u_w2 = [rows_unit(w2_hbm, w2_s, i * (R // NQ), R // NQ, 16, 1) for i in range(NQ)]
        u_t = [tail_unit(j0, nj, 128) for (j0, nj) in tail_cols]

        c_x = small(x_hbm, x_v)
        c_b1 = small(b1_hbm, b1_v)
        c_b2 = small(b2_hbm, b2_v)

        t0, t1 = [], []
        for us in (u_wq, u_k, u_v, u_wo, u_w1, u_w2):
            t0 += us[:NQ // 2]
            t1 += us[NQ // 2:]
        if cfg.get("split_tail"):
            sp = cfg["split_tail"]
            u_t = [tail_unit(j0, nj, 128, k) for (j0, nj), k in zip(tail_cols, sp)]
            u_t0 = [tail_unit(j0, nj, 128, 0, k) for (j0, nj), k in zip(tail_cols, sp)]
            t1 += u_t
            for u in t0 + t1:
                u.sem = new_sem()
            for a_, b_ in zip(u_t0, u_t):
                a_.sem = b_.sem
            t0 += [u for u in u_t0 if u.n]
        else:
            t1 += u_t
            for u in t0 + t1:
                u.sem = new_sem()
        n0 = sum(u.n for u in t0)
        n1 = sum(u.n for u in t1)
        P = n1 - n0
        assert P >= 0

        ready = {}
        pos = 0
        for u in t0:
            pos += u.n
            ready[id(u)] = pos + m0
        pos = 0
        for u in t1:
            pos += u.n
            ready[id(u)] = pos - P + m1

        def locate(lst, k):
            for u in lst:
                if k < u.n:
                    return u, k
                k -= u.n
            return None, 0

        state = {"slot": -P}

        def start(u, i, prio):
            s, d = u.piece(i)
            pltpu.make_async_copy(s, d, u.sem).start(priority=prio)

        def issue_until(slot):
            slot = min(slot, n0)
            while state["slot"] < slot:
                s = state["slot"]
                ua, ia = locate(t0, s) if s >= 0 else (None, 0)
                ub, ib = locate(t1, s + P)
                n = slot - s
                if s < 0:
                    n = min(n, -s)
                if ua is not None:
                    n = min(n, ua.n - ia)
                n = min(n, ub.n - ib)
                nl = n // UN
                if nl >= 2 and not cfg.get('static'):
                    def body(k, c, ua=ua, ia=ia, ub=ub, ib=ib):
                        for j in range(UN):
                            if ua is not None:
                                start(ua, ia + k * UN + j, 0)
                            start(ub, ib + k * UN + j, 1)
                        return c
                    jax.lax.fori_loop(0, nl, body, 0)
                    done = nl * UN
                else:
                    done = 0
                for j in range(done, n):
                    if ua is not None:
                        start(ua, ia + j, 0)
                    start(ub, ib + j, 1)
                state["slot"] = s + n

        nctr = [0]
        def need(u):
            nctr[0] += 1
            if cfg.get("scopes"):
                with jax.named_scope("iss%02d" % nctr[0]):
                    issue_until(ready[id(u)])
                s, d = u.whole()
                with jax.named_scope("wait%02d" % nctr[0]):
                    pltpu.make_async_copy(s, d, u.sem).wait()
                return
            issue_until(ready[id(u)])
            s, d = u.whole()
            pltpu.make_async_copy(s, d, u.sem).wait()

        def mm_relayout(lhs, stage, packed, r0, rc):
            w = stage[pl.ds(r0, rc), :]
            packed[pl.ds(r0 // 2, rc // 2), :] = pltpu.bitcast(w, U32)
            return _dot(lhs[:, r0:r0 + rc], w)

        def unpack(p):
            return pltpu.bitcast(p, BF16)

        def scatter_q(q):
            for h in range(Hq):
                q_scr[pl.ds(h * B, B), :] = q[:, h * Dh:(h + 1) * Dh]

        def load_qg(b, kv):
            return q_scr[pl.ds(kv * rep * B + b, rep, stride=B), :].astype(BF16)

        def softmax_pv(s, b, kv):
            m = jnp.max(s, axis=-1, keepdims=True)
            p = jnp.exp(s - m)
            l = jnp.sum(p, axis=-1, keepdims=True)
            o = _dot(p.astype(BF16), v_s[b, kv]) / l
            o_scr[pl.ds(kv * rep * B + b, rep, stride=B), :] = o

        def gather_o():
            return jnp.concatenate([o_scr[pl.ds(h * B, B), :] for h in range(Hq)], axis=1).astype(BF16)

        def bias_row(b_v, n):
            bf = b_v[...].astype(F32)
            return jnp.concatenate([bf[j:j + 1, :] for j in range(n)], axis=1)

        uorder = [0, 2, 1, 3]

        if cfg.get("dma_only"):
            issue_until(8)
            c_x.wait(); c_b1.wait(); c_b2.wait()
            for us in (u_wq, u_k, u_v, u_wo, u_w1, u_w2):
                for i in uorder:
                    need(us[i])
            issue_until(n0)
            for u in u_t:
                need(u)
            o_ref[...] = x_v[...]
            return
        if cfg.get("issue_probe") is not None:
            c_x.wait(); c_b1.wait(); c_b2.wait()
            issue_until(cfg["issue_probe"])
            w0 = jnp.zeros((1024, 1024), BF16)
            wo_p[pl.ds(0, 512), :] = pltpu.bitcast(w0, U32)
            def body(i, x):
                y = _dot(x.astype(BF16), unpack(wo_p[pl.ds(0, 512), :]))
                return x + y * 1e-6
            xx = jax.lax.fori_loop(0, cfg["R"], body, x_v[...].astype(F32))
            issue_until(n0)
            for us in (u_wq, u_k, u_v, u_wo, u_w1, u_w2, u_t):
                for u in us:
                    need(u)
            o_ref[...] = xx.astype(BF16)
            return
        issue_until(8)
        c_x.wait()
        c_b1.wait()
        c_b2.wait()
        x0 = x_v[...].astype(F32)
        lhs = _with_ones(_ln(x0))
        b1 = bias_row(b1_v, NF)
        b2 = bias_row(b2_v, ND)
        q = None
        for i in uorder:
            need(u_wq[i])
            part = mm_relayout(lhs, wq_s, wq_p, i * (D // NQ), D // NQ)
            q = part if q is None else q + part
        cs_q = q[B:B + 1, :]
        scatter_q(q[:B] * scale)

        pending_tr = []

        def do_tr(count, slots_each):
            for _ in range(count):
                if not pending_tr:
                    return
                b, kv = pending_tr.pop(0)
                if not cfg.get('notr'):
                    kt_p[b * Hkv + kv] = pltpu.bitcast(k_s[b, kv].T, U32)
                issue_until(state["slot"] + slots_each)

        bq = B // NQ
        for i in uorder:
            need(u_k[i])
            for b in range(i * bq, (i + 1) * bq):
                for kv in range(Hkv):
                    s_scr[b * Hkv + kv] = _dot_nt(load_qg(b, kv), k_s[b, kv])
                    pending_tr.append((b, kv))
            do_tr(cfg["tr_per"], cfg["tr_slots"])

        for i in uorder:
            need(u_v[i])
            for b in range(i * bq, (i + 1) * bq):
                for kv in range(Hkv):
                    softmax_pv(s_scr[b * Hkv + kv], b, kv)
            do_tr(cfg["tr_per"], cfg["tr_slots"])
        o = gather_o()
        x1 = x0
        for i in uorder:
            need(u_wo[i])
            x1 = x1 + mm_relayout(o, wo_s, wo_p, i * (HD // NQ), HD // NQ)
            do_tr(cfg["tr_per"], cfg["tr_slots"])
        do_tr(G, cfg["tr_slots"])

        lhs = _with_ones(_ln(_ln(x1)))
        pre = None
        for i in uorder:
            need(u_w1[i])
            part = mm_relayout(lhs, w1_s, w1_p, i * (D // NQ), D // NQ)
            pre = part if pre is None else pre + part
        cs_1 = pre[B:B + 1, :]
        h = jax.nn.gelu(pre[:B] + b1, approximate=True).astype(BF16)

        x2m = x1 + b2
        for i in uorder:
            need(u_w2[i])
            x2m = x2m + mm_relayout(h, w2_s, w2_p, i * (R // NQ), R // NQ)
        if not cfg.get('split_tail'):
            issue_until(n0)

        if cfg.get("stop") == "main":
            for u in u_t:
                need(u)
            o_ref[...] = x2m.astype(o_ref.dtype)
            return
        if isinstance(cfg.get("stop"), int):
            ns = cfg["stop"]
            for u in u_t[:ns]:
                need(u)
            def body(i, x):
                y = _dot(x.astype(BF16), unpack(wo_p[pl.ds(0, 512), :]))
                return x + y * 1e-6
            xx = jax.lax.fori_loop(0, cfg["R"], body, x2m)
            for u in u_t[ns:]:
                need(u)
            o_ref[...] = xx.astype(o_ref.dtype)
            return
        x2_parts = []
        qraw = None
        ht = h[:, R:]
        for (j0, nj), u in zip(tail_cols, u_t):
            need(u)
            x2c = jnp.concatenate(
                [x2m[:, j * LANE:(j + 1) * LANE] + _dot(ht, w2t[j]) for j in range(j0, j0 + nj)], axis=1)
            x2_parts.append(x2c)
            part = _dot(_hilo(x2c), unpack(wq_p[pl.ds(j0 * LANE // 2, nj * LANE // 2), :]))
            part = part[:B] + part[B:]
            qraw = part if qraw is None else qraw + part
        x2 = jnp.concatenate(x2_parts, axis=1)

        if cfg.get("stop") == "tail":
            o_ref[...] = (x2 + qraw[:, :D] + qraw[:, D:2*D] + qraw[:, 2*D:3*D] + qraw[:, 3*D:]).astype(o_ref.dtype)
            return
        m, v, _ = _stats(x2)
        rs = jax.lax.rsqrt(v + EPS)
        scatter_q((qraw - m * cs_q) * (rs * scale))
        order = [(b, kv) for kv in range(Hkv) for b in range(B)]
        sc = {}
        for i in range(G + L):
            if i < G:
                b, kv = order[i]
                sc[i] = _dot(load_qg(b, kv), unpack(kt_p[b * Hkv + kv]))
            if i >= L:
                b, kv = order[i - L]
                softmax_pv(sc.pop(i - L), b, kv)
        o = gather_o()
        x3 = x2 + _dot(o, unpack(wo_p[...]))

        pr = _dot(_hilo(x3), unpack(w1_p[...]))
        pr = pr[:B] + pr[B:]
        m1_, v1, d1 = _stats(x3)
        rs1 = jax.lax.rsqrt(v1 + EPS)
        m2, v2, _ = _stats(d1 * rs1)
        rs2 = jax.lax.rsqrt(v2 + EPS)
        a = rs1 * rs2
        pre = pr * a - (m1_ * a + m2 * rs2) * cs_1 + b1
        h = jax.nn.gelu(pre, approximate=True).astype(BF16)
        y = _dot(h[:, :R], unpack(w2_p[...]))
        ht = h[:, R:]
        yt = jnp.concatenate([_dot(ht, w2t[j]) for j in range(ND)], axis=1)
        x4 = x3 + b2 + y + yt
        o_ref[...] = x4.astype(o_ref.dtype)

    scratch = [
        pltpu.VMEM((B, D), BF16), pltpu.VMEM((NF, LANE), BF16), pltpu.VMEM((ND, LANE), BF16),
        pltpu.VMEM((D, HD), BF16), pltpu.VMEM((B, Hkv, W, Dh), BF16), pltpu.VMEM((B, Hkv, W, Dh), BF16),
        pltpu.VMEM((HD, D), BF16), pltpu.VMEM((D, F), BF16), pltpu.VMEM((R, D), BF16),
        pltpu.VMEM((ND, T, LANE), BF16),
        pltpu.VMEM((D // 2, HD), U32), pltpu.VMEM((G, Dh // 2, W), U32), pltpu.VMEM((HD // 2, D), U32),
        pltpu.VMEM((D // 2, F), U32), pltpu.VMEM((R // 2, D), U32),
        pltpu.VMEM((Hq * B, Dh), F32), pltpu.VMEM((Hq * B, Dh), F32), pltpu.VMEM((G, rep, W), F32),
        pltpu.SemaphoreType.DMA((n_sems,)),
    ]
    return kernel, scratch


DEFAULT_CFG = dict(lag=4, unroll=4, margin0=34, margin1=62, tail_rows=1536, tr_per=3, tr_slots=6,
                   static=1, split_tail=(6, 5, 0, 0),
                   tail_cols=((0, 4), (4, 2), (6, 1), (7, 1)))


def build(cfg=None):
    cfg = dict(DEFAULT_CFG, **(cfg or {}))

    @jax.jit
    def fn(A_x, A_k_cache, A_v_cache, A_wq, A_wo, B_x, B_w1, B_b1, B_w2, B_b2):
        B, Sq, D = A_x.shape
        Hq, Dh = 32, 128
        Hkv, Sk = A_k_cache.shape[1], A_k_cache.shape[2]
        W = min(4096, max(256, Sk // 4))
        F = B_w1.shape[1]
        kernel, scratch = make_kernel(B, D, Hq, Hkv, Sk, Dh, F, W, cfg)
        any_spec = pl.BlockSpec(memory_space=pl.ANY)
        out = pl.pallas_call(
            kernel,
            out_shape=jax.ShapeDtypeStruct((B, D), A_x.dtype),
            in_specs=[any_spec] * 9,
            out_specs=pl.BlockSpec(memory_space=pltpu.VMEM),
            scratch_shapes=scratch,
            compiler_params=pltpu.CompilerParams(
                vmem_limit_bytes=110 * 1024 * 1024,
                disable_semaphore_checks=True,
                disable_bounds_checks=bool(cfg.get('nobc'))),
        )(A_x.reshape(B, D), A_k_cache, A_v_cache, A_wq, A_wo, B_w1,
          B_b1.reshape(F // LANE, LANE), B_w2, B_b2.reshape(D // LANE, LANE))
        return out.reshape(B, Sq, D)

    return fn


pallas_interleave_layers__sliding_block_cached__mixer_channel_mlp__decode_kernel = build()
```

```python
import math

import jax
import jax.numpy as jnp
import jax.experimental.pallas as pl
import jax.experimental.pallas.tpu as pltpu

F32 = jnp.float32
BF16 = jnp.bfloat16
U32 = jnp.uint32
EPS = 1e-5
LANE = 128
LOG2E = math.log2(math.e)


def _stats(x):
    m = jnp.mean(x, axis=-1, keepdims=True)
    d = x - m
    v = jnp.mean(d * d, axis=-1, keepdims=True)
    return m, v, d


def _ln(x):
    _, v, d = _stats(x)
    return d * jax.lax.rsqrt(v + EPS)


def _hilo(x):
    hi = x.astype(BF16).astype(F32)
    return jnp.concatenate([hi, x - hi], axis=0).astype(BF16)


def _with_ones(x):
    r = jax.lax.broadcasted_iota(jnp.int32, x.shape, 0)
    ones = jnp.where(r == 0, 1.0, 0.0).astype(F32)
    return jnp.concatenate([x, ones], axis=0).astype(BF16)


def _dot(a, b):
    return jnp.dot(a, b, preferred_element_type=F32)


def _dot_nt(a, b):
    return jax.lax.dot_general(a, b, (((1,), (1,)), ((), ())), preferred_element_type=F32)


def _splits(total, step):
    out, r = [], 0
    while r < total:
        p = min(step, total - r)
        out.append((r, p))
        r += p
    return out


class _Unit:
    def __init__(self, whole):
        self.whole = whole
        self.sem = None
        self.ready = 0


def make_kernel(B, D, Hq, Hkv, Sk, Dh, F, W, cfg):
    rep = Hq // Hkv
    G = B * Hkv
    HD = Hq * Dh
    T = cfg["tail_rows"]
    R = F - T
    tail = cfg["tail"]
    scale = Dh ** -0.5
    NF = F // LANE
    ND = D // LANE
    L = cfg["lag"]
    lag_slots = (cfg["margin0"], cfg["margin1"])
    NQ = 4
    n_sems = 3 + 6 * NQ + len(tail)

    def kernel(x_hbm, k_hbm, v_hbm, wq_hbm, wo_hbm, w1_hbm, b1_hbm, w2_hbm, b2_hbm,
               o_ref,
               x_v, b1_v, b2_v,
               wq_s, k_s, v_s, wo_s, w1_s, w2_s, w2t,
               wq_p, kt_p, wo_p, w1_p, w2_p,
               q_scr, o_scr, s_scr,
               sems, bar):
        n_used = [0]

        def barrier():
            if cfg.get('bar'):
                pl.semaphore_signal(bar, 1)
                pl.semaphore_wait(bar, 1)


        def new_sem():
            s = sems.at[n_used[0]]
            n_used[0] += 1
            return s

        def small(src, dst):
            c = pltpu.make_async_copy(src, dst, new_sem())
            c.start(priority=0)
            return c

        if not cfg.get('late_small'):
            c_x = small(x_hbm, x_v)
            c_b1 = small(b1_hbm, b1_v)
            c_b2 = small(b2_hbm, b2_v)

        streams = ([], [])

        def new_unit(whole):
            u = _Unit(whole)
            u.sem = new_sem()
            return u

        def rows_unit(hbm, stage, r0, rc, prow, ncol, th):
            u = new_unit(stage.at[pl.ds(r0, rc)])
            cw = hbm.shape[1] // ncol
            for r, p in _splits(rc, prow):
                for c in range(ncol):
                    idx = (pl.ds(r0 + r, p), pl.ds(c * cw, cw))
                    streams[th].append((hbm.at[idx], stage.at[idx], u))
            return u

        def kv_unit(hbm, stage, b0, nb, prow, th):
            u = new_unit(stage.at[pl.ds(b0, nb)])
            for b in range(b0, b0 + nb):
                for kv in range(Hkv):
                    for r, p in _splits(W, prow):
                        streams[th].append((hbm.at[b, kv, pl.ds(Sk - W + r, p), :],
                                            stage.at[b, kv, pl.ds(r, p), :], u))
            return u

        def tail_unit(j0, nj, row0, nrows, n0):
            u = new_unit(w2t.at[pl.ds(j0, nj), pl.ds(row0, nrows)])
            for i, (r, p) in enumerate(_splits(nrows, cfg["tail_prow"])):
                for j in range(j0, j0 + nj):
                    streams[0 if i < n0 else 1].append(
                        (w2_hbm.at[pl.ds(R + row0 + r, p), pl.ds(j * LANE, LANE)],
                         w2t.at[j, pl.ds(row0 + r, p), :], u))
            return u

        th = [0, 0, 1, 1]
        u_wq = [rows_unit(wq_hbm, wq_s, i * (D // NQ), D // NQ, 8, 2, th[i]) for i in range(NQ)]
        u_k = [kv_unit(k_hbm, k_s, i * (B // NQ), B // NQ, cfg["kv_prow"], th[i]) for i in range(NQ)]
        u_v = [kv_unit(v_hbm, v_s, i * (B // NQ), B // NQ, cfg["kv_prow"], th[i]) for i in range(NQ)]
        u_wo = [rows_unit(wo_hbm, wo_s, i * (HD // NQ), HD // NQ, cfg["wo_prow"], 1, th[i]) for i in range(NQ)]
        u_w1 = [rows_unit(w1_hbm, w1_s, i * (D // NQ), D // NQ, 8, cfg["w1_ncol"], th[i]) for i in range(NQ)]
        u_w2 = [rows_unit(w2_hbm, w2_s, i * (R // NQ), R // NQ, cfg["wo_prow"], 1, th[i]) for i in range(NQ)]
        u_t = [tail_unit(*t) for t in tail]

        n_slots = len(streams[0])
        lead = len(streams[1]) - n_slots
        assert lead >= 0
        for i, (_, _, u) in enumerate(streams[0]):
            u.ready = max(u.ready, i + 1 + lag_slots[0])
        for i, (_, _, u) in enumerate(streams[1]):
            u.ready = max(u.ready, i + 1 - lead + lag_slots[1])

        cur = [-lead]

        def issue_until(slot):
            while cur[0] < min(slot, n_slots):
                s = cur[0]
                if s >= 0:
                    src, dst, u = streams[0][s]
                    pltpu.make_async_copy(src, dst, u.sem).start(priority=0)
                src, dst, u = streams[1][s + lead]
                pltpu.make_async_copy(src, dst, u.sem).start(priority=1)
                cur[0] += 1

        if cfg.get('late_small'):
            issue_until(-lead + cfg['late_small'])
            c_x = small(x_hbm, x_v)
            c_b1 = small(b1_hbm, b1_v)
            c_b2 = small(b2_hbm, b2_v)

        nctr = [0]

        def need(u):
            nctr[0] += 1
            if cfg.get("scopes") and nctr[0] >= cfg.get("scope_from", 0) and nctr[0] < cfg.get("scope_to", 99):
                with jax.named_scope("iss%02d" % nctr[0]):
                    issue_until(u.ready)
                with jax.named_scope("wait%02d" % nctr[0]):
                    pltpu.make_async_copy(u.whole, u.whole, u.sem).wait()
                return
            if cur[0] < min(u.ready, n_slots):
                barrier()
            issue_until(u.ready)
            pltpu.make_async_copy(u.whole, u.whole, u.sem).wait()

        def mm_relayout(lhs, stage, packed, r0, rc):
            w = stage[pl.ds(r0, rc), :]
            packed[pl.ds(r0 // 2, rc // 2), :] = pltpu.bitcast(w, U32)
            return _dot(lhs[:, r0:r0 + rc], w)

        def unpack(p):
            return pltpu.bitcast(p, BF16)

        def scatter_q(q):
            for h in range(Hq):
                q_scr[pl.ds(h * B, B), :] = q[:, h * Dh:(h + 1) * Dh]

        def load_qg(b, kv):
            return q_scr[pl.ds(kv * rep * B + b, rep, stride=B), :].astype(BF16)

        def softmax_pv(s, b, kv, c):
            m = jnp.max(s, axis=-1, keepdims=True)
            p = jnp.exp2((s - m) * c)
            l = jnp.sum(p, axis=-1, keepdims=True)
            o = _dot(p.astype(BF16), v_s[b, kv]) / l
            o_scr[pl.ds(kv * rep * B + b, rep, stride=B), :] = o

        def gather_o():
            return jnp.concatenate([o_scr[pl.ds(h * B, B), :] for h in range(Hq)], axis=1).astype(BF16)

        def bias_row(b_v, n):
            bf = b_v[...].astype(F32)
            return jnp.concatenate([bf[j:j + 1, :] for j in range(n)], axis=1)

        uorder = [0, 2, 1, 3]

        if cfg.get("dma_only"):
            issue_until(8)
            c_x.wait(); c_b1.wait(); c_b2.wait()
            for us in (u_wq, u_k, u_v, u_wo, u_w1, u_w2):
                for i in uorder:
                    need(us[i])
            for u in u_t:
                need(u)
            o_ref[...] = x_v[...]
            return

        issue_until(cfg.get('first', 8))
        c_x.wait()
        c_b1.wait()
        c_b2.wait()
        x0 = x_v[...].astype(F32)
        lhs = _with_ones(_ln(x0))
        b1 = bias_row(b1_v, NF)
        b2 = bias_row(b2_v, ND)
        q = None
        for i in uorder:
            need(u_wq[i])
            part = mm_relayout(lhs, wq_s, wq_p, i * (D // NQ), D // NQ)
            q = part if q is None else part + q
        cs_q = q[B:B + 1, :]
        scatter_q(q[:B])

        pending_tr = []

        def do_tr(count):
            for _ in range(count):
                if not pending_tr:
                    return
                b, kv = pending_tr.pop(0)
                kt_p[b * Hkv + kv] = pltpu.bitcast(k_s[b, kv].T, U32)
                if cfg.get('bar') == 2:
                    barrier()
                issue_until(cur[0] + cfg["tr_slots"])
                if cfg.get('bar') == 2:
                    barrier()

        bq = B // NQ
        for i in uorder:
            need(u_k[i])
            for b in range(i * bq, (i + 1) * bq):
                for kv in range(Hkv):
                    s_scr[b * Hkv + kv] = _dot_nt(load_qg(b, kv), k_s[b, kv])
                    pending_tr.append((b, kv))
            do_tr(cfg["tr_per"])

        for i in uorder:
            need(u_v[i])
            for b in range(i * bq, (i + 1) * bq):
                for kv in range(Hkv):
                    softmax_pv(s_scr[b * Hkv + kv], b, kv, scale * LOG2E)
            do_tr(cfg["tr_per"])
        o = gather_o()
        x1 = x0
        for i in uorder:
            need(u_wo[i])
            x1 = x1 + mm_relayout(o, wo_s, wo_p, i * (HD // NQ), HD // NQ)
            do_tr(cfg["tr_per"])
        do_tr(G)

        lhs = _with_ones(_ln(_ln(x1)))
        pre = None
        for i in uorder:
            need(u_w1[i])
            part = mm_relayout(lhs, w1_s, w1_p, i * (D // NQ), D // NQ)
            pre = part if pre is None else part + pre
        cs_1 = pre[B:B + 1, :]
        h = jax.nn.gelu(pre[:B] + b1, approximate=True).astype(BF16)

        x2m = x1 + b2
        for i in uorder:
            need(u_w2[i])
            x2m = x2m + mm_relayout(h, w2_s, w2_p, i * (R // NQ), R // NQ)

        x2b = [x2m[:, j * LANE:(j + 1) * LANE] for j in range(ND)]
        rows_done = [0] * ND
        qraw = None
        for (j0, nj, row0, nrows, _), u in zip(tail, u_t):
            need(u)
            ht = h[:, R + row0:R + row0 + nrows]
            for j in range(j0, j0 + nj):
                x2b[j] = x2b[j] + _dot(ht, w2t[j, pl.ds(row0, nrows), :])
                rows_done[j] += nrows
            if rows_done[j0] == T:
                x2c = jnp.concatenate(x2b[j0:j0 + nj], axis=1)
                part = _dot(_hilo(x2c), unpack(wq_p[pl.ds(j0 * LANE // 2, nj * LANE // 2), :]))
                part = part[:B] + part[B:]
                qraw = part if qraw is None else qraw + part
        assert all(r == T for r in rows_done)
        x2 = jnp.concatenate(x2b, axis=1)

        m, v, _ = _stats(x2)
        cexp = jax.lax.rsqrt(v + EPS) * (scale * LOG2E)
        scatter_q(qraw - m * cs_q)
        order = [(b, kv) for kv in range(Hkv) for b in range(B)]
        sc = {}
        for i in range(G + L):
            if i < G:
                b, kv = order[i]
                sc[i] = _dot(load_qg(b, kv), unpack(kt_p[b * Hkv + kv]))
            if i >= L:
                b, kv = order[i - L]
                softmax_pv(sc.pop(i - L), b, kv, cexp[b:b + 1, :])
        o = gather_o()
        x3 = x2 + _dot(o, unpack(wo_p[...]))

        pr = _dot(_hilo(x3), unpack(w1_p[...]))
        pr = pr[:B] + pr[B:]
        m1, v1, d1 = _stats(x3)
        rs1 = jax.lax.rsqrt(v1 + EPS)
        m2, v2, _ = _stats(d1 * rs1)
        rs2 = jax.lax.rsqrt(v2 + EPS)
        a = rs1 * rs2
        pre = pr * a - (m1 * a + m2 * rs2) * cs_1 + b1
        h = jax.nn.gelu(pre, approximate=True).astype(BF16)
        y = _dot(h[:, :R], unpack(w2_p[...]))
        ht = h[:, R:]
        yt = jnp.concatenate([_dot(ht, w2t[j]) for j in range(ND)], axis=1)
        x4 = x3 + b2 + y + yt
        o_ref[...] = x4.astype(o_ref.dtype)
        if cfg.get("scopes"):
            with jax.named_scope("endmark"):
                q_scr[pl.ds(0, 8), :] = x4[:, :LANE]

    scratch = [
        pltpu.VMEM((B, D), BF16), pltpu.VMEM((NF, LANE), BF16), pltpu.VMEM((ND, LANE), BF16),
        pltpu.VMEM((D, HD), BF16), pltpu.VMEM((B, Hkv, W, Dh), BF16), pltpu.VMEM((B, Hkv, W, Dh), BF16),
        pltpu.VMEM((HD, D), BF16), pltpu.VMEM((D, F), BF16), pltpu.VMEM((R, D), BF16),
        pltpu.VMEM((ND, T, LANE), BF16),
        pltpu.VMEM((D // 2, HD), U32), pltpu.VMEM((G, Dh // 2, W), U32), pltpu.VMEM((HD // 2, D), U32),
        pltpu.VMEM((D // 2, F), U32), pltpu.VMEM((R // 2, D), U32),
        pltpu.VMEM((Hq * B, Dh), F32), pltpu.VMEM((Hq * B, Dh), F32), pltpu.VMEM((G, rep, W), F32),
        pltpu.SemaphoreType.DMA((n_sems,)), pltpu.SemaphoreType.REGULAR,
    ]
    return kernel, scratch


DEFAULT_CFG = dict(lag=4, margin0=34, margin1=62, tail_rows=1536, tr_per=4, tr_slots=0, bar=1,
                   kv_prow=176, wo_prow=24, w1_ncol=1, tail_prow=128,
                   tail=((0, 2, 0, 1536, 6), (2, 2, 0, 1536, 6), (4, 2, 0, 1536, 5),
                         (6, 1, 0, 1536, 0), (7, 1, 0, 1536, 0)))


def build(cfg=None):
    cfg = dict(DEFAULT_CFG, **(cfg or {}))

    @jax.jit
    def fn(A_x, A_k_cache, A_v_cache, A_wq, A_wo, B_x, B_w1, B_b1, B_w2, B_b2):
        B, Sq, D = A_x.shape
        Hq, Dh = 32, 128
        Hkv, Sk = A_k_cache.shape[1], A_k_cache.shape[2]
        W = min(4096, max(256, Sk // 4))
        F = B_w1.shape[1]
        kernel, scratch = make_kernel(B, D, Hq, Hkv, Sk, Dh, F, W, cfg)
        any_spec = pl.BlockSpec(memory_space=pl.ANY)
        out = pl.pallas_call(
            kernel,
            out_shape=jax.ShapeDtypeStruct((B, D), A_x.dtype),
            in_specs=[any_spec] * 9,
            out_specs=pl.BlockSpec(memory_space=pltpu.VMEM),
            scratch_shapes=scratch,
            compiler_params=pltpu.CompilerParams(
                vmem_limit_bytes=110 * 1024 * 1024,
                disable_semaphore_checks=True),
        )(A_x.reshape(B, D), A_k_cache, A_v_cache, A_wq, A_wo, B_w1,
          B_b1.reshape(F // LANE, LANE), B_w2, B_b2.reshape(D // LANE, LANE))
        return out.reshape(B, Sq, D)

    return fn


pallas_interleave_layers__sliding_block_cached__mixer_channel_mlp__decode_kernel = build()
```

```python
import math

import jax
import jax.numpy as jnp
import jax.experimental.pallas as pl
import jax.experimental.pallas.tpu as pltpu

F32 = jnp.float32
BF16 = jnp.bfloat16
U32 = jnp.uint32
EPS = 1e-5
LANE = 128
LOG2E = math.log2(math.e)


def _stats(x):
    m = jnp.mean(x, axis=-1, keepdims=True)
    d = x - m
    v = jnp.mean(d * d, axis=-1, keepdims=True)
    return m, v, d


def _ln(x):
    _, v, d = _stats(x)
    return d * jax.lax.rsqrt(v + EPS)


def _hilo(x):
    hi = x.astype(BF16).astype(F32)
    return jnp.concatenate([hi, x - hi], axis=0).astype(BF16)


def _with_ones(x):
    r = jax.lax.broadcasted_iota(jnp.int32, x.shape, 0)
    ones = jnp.where(r == 0, 1.0, 0.0).astype(F32)
    return jnp.concatenate([x, ones], axis=0).astype(BF16)


def _dot(a, b):
    return jnp.dot(a, b, preferred_element_type=F32)


def _dot_nt(a, b):
    return jax.lax.dot_general(a, b, (((1,), (1,)), ((), ())), preferred_element_type=F32)


def _splits(total, step):
    out, r = [], 0
    while r < total:
        p = min(step, total - r)
        out.append((r, p))
        r += p
    return out


class _Unit:
    def __init__(self, whole):
        self.whole = whole
        self.sem = None
        self.ready = 0


def make_kernel(B, D, Hq, Hkv, Sk, Dh, F, W, cfg):
    rep = Hq // Hkv
    G = B * Hkv
    HD = Hq * Dh
    T = cfg["tail_rows"]
    R = F - T
    tail = cfg["tail"]
    scale = Dh ** -0.5
    NF = F // LANE
    ND = D // LANE
    L = cfg["lag"]
    lag_slots = (cfg["margin0"], cfg["margin1"])
    NQ, NKV, NW2 = cfg['nq'], cfg['nkv'], cfg['nw2']
    NS = cfg['ns']
    NS2 = cfg['ns2']
    RS = R // (2 * NS2)
    SL = RS // NW2
    n_sems = 3 + 3 * NQ + 2 * NKV + NW2 + len(tail)

    def kernel(x_hbm, k_hbm, v_hbm, wq_hbm, wo_hbm, w1_hbm, b1_hbm, w2_hbm, b2_hbm,
               o_ref,
               x_v, b1_v, b2_v,
               wq_s, k_s, v_s, wo_s, w1_s, w2_s, w2t,
               wq_p, kt_p, wo_p, w1_p, w2_p,
               q_scr, o_scr, s_scr,
               sems, bar):
        n_used = [0]

        def barrier():
            if cfg.get('bar'):
                pl.semaphore_signal(bar, 1)
                pl.semaphore_wait(bar, 1)


        def new_sem():
            s = sems.at[n_used[0]]
            n_used[0] += 1
            return s

        def small(src, dst):
            c = pltpu.make_async_copy(src, dst, new_sem())
            c.start(priority=0)
            return c

        if not cfg.get('late_small'):
            c_x = small(x_hbm, x_v)
            c_b1 = small(b1_hbm, b1_v)
            c_b2 = small(b2_hbm, b2_v)

        streams = ([], [])

        def new_unit(whole):
            u = _Unit(whole)
            u.sem = new_sem()
            return u


        def add_region(blocks, u):
            n, k = len(blocks), 2 * NS
            subs = [blocks[n * i // k:n * (i + 1) // k] for i in range(k)]
            for t in range(2):
                ss = subs[t * NS:(t + 1) * NS]
                for i in range(max(len(x) for x in ss)):
                    for x in ss:
                        if i < len(x):
                            streams[t].append((x[i], u))

        def tile_blocks(t0, t1, off):
            cuts = [t0] + [t for t in range(t0 + 1, t1) if (t - off) % 16 == 0] + [t1]
            return list(zip(cuts[:-1], cuts[1:]))

        def rows_unit(hbm, stage, r0, rc, off):
            u = new_unit(stage.at[pl.ds(r0, rc)])
            nt = hbm.shape[1] // LANE
            blocks = []
            for a, b in tile_blocks(r0 // 8 * nt, (r0 + rc) // 8 * nt, off):
                blk = []
                while a < b:
                    g, j = divmod(a, nt)
                    if j == 0 and b - a >= nt:
                        ng = (b - a) // nt
                        idx = (pl.ds(g * 8, ng * 8),)
                        a += ng * nt
                    else:
                        e = min(b - g * nt, nt)
                        idx = (pl.ds(g * 8, 8), pl.ds(j * LANE, (e - j) * LANE))
                        a = g * nt + e
                    blk.append((hbm.at[idx], stage.at[idx]))
                blocks.append(blk)
            add_region(blocks, u)
            return u

        def kv_unit(hbm, stage, b0, nb, off):
            u = new_unit(stage.at[pl.ds(b0, nb)])
            blocks = []
            for b in range(b0, b0 + nb):
                for kv in range(Hkv):
                    for a, e in tile_blocks(0, W // 8, off):
                        blocks.append([(hbm.at[b, kv, pl.ds(Sk - W + a * 8, (e - a) * 8), :],
                                        stage.at[b, kv, pl.ds(a * 8, (e - a) * 8), :])])
            add_region(blocks, u)
            return u

        def tail_unit(j0, nj, row0, nrows, n0):
            u = new_unit(w2t.at[pl.ds(j0, nj), pl.ds(row0, nrows)])
            for i, (r, p) in enumerate(_splits(nrows, cfg["tail_prow"])):
                for j in range(j0, j0 + nj):
                    streams[0 if i < n0 else 1].append(
                        ([(w2_hbm.at[pl.ds(R + row0 + r, p), pl.ds(j * LANE, LANE)],
                           w2t.at[j, pl.ds(row0 + r, p), :])], u))
            return u

        offs = cfg["offs"]
        u_wq = [rows_unit(wq_hbm, wq_s, i * (D // NQ), D // NQ, offs[2]) for i in range(NQ)]
        u_k = [kv_unit(k_hbm, k_s, i * (B // NKV), B // NKV, offs[0]) for i in range(NKV)]
        u_v = [kv_unit(v_hbm, v_s, i * (B // NKV), B // NKV, offs[1]) for i in range(NKV)]
        u_wo = [rows_unit(wo_hbm, wo_s, i * (HD // NQ), HD // NQ, offs[3]) for i in range(NQ)]
        u_w1 = [rows_unit(w1_hbm, w1_s, i * (D // NQ), D // NQ, offs[4]) for i in range(NQ)]
        u_w2 = []
        for i in range(NW2):
            u = new_unit(w2_s.at[:, pl.ds(i * SL, SL)])
            u_w2.append(u)
            for r, p in _splits(SL, 16):
                for s in range(2 * NS2):
                    streams[s // NS2].append(
                        ([(w2_hbm.at[pl.ds(s * RS + i * SL + r, p)], w2_s.at[s, pl.ds(i * SL + r, p)])], u))
        u_t = [tail_unit(*t) for t in tail]

        n_slots = len(streams[0])
        lead = len(streams[1]) - n_slots
        assert lead >= 0
        late = cfg["late"]
        for u in u_wq + u_k + u_v + u_wo + u_w1 + u_t:
            u.cut = 0
        for u, c in zip(u_w2, late):
            u.cut = c
        for i, (_, u) in enumerate(streams[0]):
            u.ready = max(u.ready, i + 1 + lag_slots[0] - u.cut)
        for i, (_, u) in enumerate(streams[1]):
            u.ready = max(u.ready, i + 1 - lead + lag_slots[1] - u.cut)

        cur = [-lead]

        def issue_until(slot):
            while cur[0] < min(slot, n_slots):
                s = cur[0]
                for t, i in ((0, s), (1, s + lead)):
                    if i >= 0:
                        blk, u = streams[t][i]
                        for src, dst in blk:
                            pltpu.make_async_copy(src, dst, u.sem).start(priority=t)
                cur[0] += 1

        if cfg.get('late_small'):
            issue_until(-lead + cfg['late_small'])
            c_x = small(x_hbm, x_v)
            c_b1 = small(b1_hbm, b1_v)
            c_b2 = small(b2_hbm, b2_v)

        nctr = [0]

        def need(u):
            nctr[0] += 1
            if cfg.get("scopes") and nctr[0] >= cfg.get("scope_from", 0) and nctr[0] < cfg.get("scope_to", 99):
                with jax.named_scope("iss%02d" % nctr[0]):
                    issue_until(u.ready)
                with jax.named_scope("wait%02d" % nctr[0]):
                    pltpu.make_async_copy(u.whole, u.whole, u.sem).wait()
                return
            if cur[0] < min(u.ready, n_slots):
                barrier()
            issue_until(u.ready)
            pltpu.make_async_copy(u.whole, u.whole, u.sem).wait()

        def gap():
            if cfg["gap"] and cur[0] < n_slots:
                barrier()
                issue_until(cur[0] + cfg["gap"])
                barrier()

        def mm_relayout(acc, lhs, stage, packed, r0, rc):
            ns = cfg["nsub"]
            for r, p in _splits(rc, rc // ns):
                if r:
                    gap()
                w = stage[pl.ds(r0 + r, p), :]
                packed[pl.ds((r0 + r) // 2, p // 2), :] = pltpu.bitcast(w, U32)
                part = _dot(lhs[:, r0 + r:r0 + r + p], w)
                acc = part if acc is None else part + acc
            return acc

        def unpack(p):
            return pltpu.bitcast(p, BF16)

        def scatter_q(q):
            for h in range(Hq):
                q_scr[pl.ds(h * B, B), :] = q[:, h * Dh:(h + 1) * Dh]

        def load_qg(b, kv):
            return q_scr[pl.ds(kv * rep * B + b, rep, stride=B), :].astype(BF16)

        def softmax_pv(s, b, kv, c):
            m = jnp.max(s, axis=-1, keepdims=True)
            p = jnp.exp2((s - m) * c)
            l = jnp.sum(p, axis=-1, keepdims=True)
            o = _dot(p.astype(BF16), v_s[b, kv]) / l
            o_scr[pl.ds(kv * rep * B + b, rep, stride=B), :] = o

        def gather_o():
            return jnp.concatenate([o_scr[pl.ds(h * B, B), :] for h in range(Hq)], axis=1).astype(BF16)

        def bias_row(b_v, n):
            bf = b_v[...].astype(F32)
            return jnp.concatenate([bf[j:j + 1, :] for j in range(n)], axis=1)


        if cfg.get("dma_only"):
            issue_until(8)
            c_x.wait(); c_b1.wait(); c_b2.wait()
            for us in (u_wq, u_k, u_v, u_wo, u_w1, u_w2):
                for u in us:
                    need(u)
            for u in u_t:
                need(u)
            o_ref[...] = x_v[...]
            return

        issue_until(cfg.get('first', 8))
        c_x.wait()
        c_b1.wait()
        c_b2.wait()
        x0 = x_v[...].astype(F32)
        lhs = _with_ones(_ln(x0))
        b1 = bias_row(b1_v, NF)
        b2 = bias_row(b2_v, ND)
        q = None
        for i in range(NQ):
            need(u_wq[i])
            q = mm_relayout(q, lhs, wq_s, wq_p, i * (D // NQ), D // NQ)
        cs_q = q[B:B + 1, :]
        scatter_q(q[:B])

        pending_tr = []

        def do_tr(count):
            for n in range(count):
                if not pending_tr:
                    return
                if n % cfg["tr_grp"] == 0 and cfg["tr_gap"]:
                    gap()
                b, kv = pending_tr.pop(0)
                kt_p[b * Hkv + kv] = pltpu.bitcast(k_s[b, kv].T, U32)

        bq = B // NKV
        for i in range(NKV):
            need(u_k[i])
            for b in range(i * bq, (i + 1) * bq):
                if b > i * bq and (b - i * bq) % cfg["b_grp"] == 0:
                    gap()
                for kv in range(Hkv):
                    s_scr[b * Hkv + kv] = _dot_nt(load_qg(b, kv), k_s[b, kv])
                    pending_tr.append((b, kv))
            do_tr(cfg["tr_per"])

        for i in range(NKV):
            need(u_v[i])
            for b in range(i * bq, (i + 1) * bq):
                if b > i * bq and (b - i * bq) % (2 * cfg["b_grp"]) == 0:
                    gap()
                for kv in range(Hkv):
                    softmax_pv(s_scr[b * Hkv + kv], b, kv, scale * LOG2E)
            do_tr(cfg["tr_per"])
        o = gather_o()
        x1 = x0
        for i in range(NQ):
            need(u_wo[i])
            x1 = mm_relayout(x1, o, wo_s, wo_p, i * (HD // NQ), HD // NQ)
            do_tr(cfg["tr_per"])
        do_tr(G)

        lhs = _with_ones(_ln(_ln(x1)))
        pre = None
        for i in range(NQ):
            need(u_w1[i])
            pre = mm_relayout(pre, lhs, w1_s, w1_p, i * (D // NQ), D // NQ)
        cs_1 = pre[B:B + 1, :]
        h = jax.nn.gelu(pre[:B] + b1, approximate=True).astype(BF16)

        x2m = x1 + b2
        for i in range(NW2):
            need(u_w2[i])
            w = w2_s[:, pl.ds(i * SL, SL), :]
            w2_p[:, pl.ds(i * SL // 2, SL // 2), :] = pltpu.bitcast(w, U32)
            hs = jnp.concatenate([h[:, s * RS + i * SL:s * RS + (i + 1) * SL] for s in range(2 * NS2)], axis=1)
            x2m = x2m + _dot(hs, w.reshape(2 * NS2 * SL, D))

        x2b = [x2m[:, j * LANE:(j + 1) * LANE] for j in range(ND)]
        rows_done = [0] * ND
        qraw = None
        for (j0, nj, row0, nrows, _), u in zip(tail, u_t):
            need(u)
            ht = h[:, R + row0:R + row0 + nrows]
            for j in range(j0, j0 + nj):
                x2b[j] = x2b[j] + _dot(ht, w2t[j, pl.ds(row0, nrows), :])
                rows_done[j] += nrows
            if rows_done[j0] == T:
                x2c = jnp.concatenate(x2b[j0:j0 + nj], axis=1)
                part = _dot(_hilo(x2c), unpack(wq_p[pl.ds(j0 * LANE // 2, nj * LANE // 2), :]))
                part = part[:B] + part[B:]
                qraw = part if qraw is None else qraw + part
        assert all(r == T for r in rows_done)
        x2 = jnp.concatenate(x2b, axis=1)

        m, v, _ = _stats(x2)
        cexp = jax.lax.rsqrt(v + EPS) * (scale * LOG2E)
        scatter_q(qraw - m * cs_q)
        order = [(b, kv) for kv in range(Hkv) for b in range(B)]
        sc = {}
        for i in range(G + L):
            if i < G:
                b, kv = order[i]
                sc[i] = _dot(load_qg(b, kv), unpack(kt_p[b * Hkv + kv]))
            if i >= L:
                b, kv = order[i - L]
                softmax_pv(sc.pop(i - L), b, kv, cexp[b:b + 1, :])
        o = gather_o()
        x3 = x2 + _dot(o, unpack(wo_p[...]))

        pr = _dot(_hilo(x3), unpack(w1_p[...]))
        pr = pr[:B] + pr[B:]
        m1, v1, d1 = _stats(x3)
        rs1 = jax.lax.rsqrt(v1 + EPS)
        m2, v2, _ = _stats(d1 * rs1)
        rs2 = jax.lax.rsqrt(v2 + EPS)
        a = rs1 * rs2
        pre = pr * a - (m1 * a + m2 * rs2) * cs_1 + b1
        h = jax.nn.gelu(pre, approximate=True).astype(BF16)
        y = _dot(h[:, :R], unpack(w2_p[...].reshape(R // 2, D)))
        ht = h[:, R:]
        yt = jnp.concatenate([_dot(ht, w2t[j]) for j in range(ND)], axis=1)
        x4 = x3 + b2 + y + yt
        o_ref[...] = x4.astype(o_ref.dtype)
        if cfg.get("scopes"):
            with jax.named_scope("endmark"):
                q_scr[pl.ds(0, 8), :] = x4[:, :LANE]

    scratch = [
        pltpu.VMEM((B, D), BF16), pltpu.VMEM((NF, LANE), BF16), pltpu.VMEM((ND, LANE), BF16),
        pltpu.VMEM((D, HD), BF16), pltpu.VMEM((B, Hkv, W, Dh), BF16), pltpu.VMEM((B, Hkv, W, Dh), BF16),
        pltpu.VMEM((HD, D), BF16), pltpu.VMEM((D, F), BF16), pltpu.VMEM((2 * NS2, RS, D), BF16),
        pltpu.VMEM((ND, T, LANE), BF16),
        pltpu.VMEM((D // 2, HD), U32), pltpu.VMEM((G, Dh // 2, W), U32), pltpu.VMEM((HD // 2, D), U32),
        pltpu.VMEM((D // 2, F), U32), pltpu.VMEM((2 * NS2, RS // 2, D), U32),
        pltpu.VMEM((Hq * B, Dh), F32), pltpu.VMEM((Hq * B, Dh), F32), pltpu.VMEM((G, rep, W), F32),
        pltpu.SemaphoreType.DMA((n_sems,)), pltpu.SemaphoreType.REGULAR,
    ]
    return kernel, scratch


DEFAULT_CFG = dict(b_grp=2, gap=10, nsub=2, tr_grp=3, tr_gap=1, late=(0, 0), lag=4, margin0=34, margin1=62,
                   tail_rows=1536, tr_per=6, bar=1,
                   ns2=4, offs=(5, 5, 5, 5, 13, 0), tail_prow=128, ns=4, nq=2, nkv=2, nw2=2,
                   tail=((0, 2, 0, 1536, 6), (2, 2, 0, 1536, 6), (4, 1, 0, 1536, 6), (5, 1, 0, 1536, 4),
                         (6, 1, 0, 1536, 0), (7, 1, 0, 1536, 0)))


def build(cfg=None):
    cfg = dict(DEFAULT_CFG, **(cfg or {}))

    @jax.jit
    def fn(A_x, A_k_cache, A_v_cache, A_wq, A_wo, B_x, B_w1, B_b1, B_w2, B_b2):
        B, Sq, D = A_x.shape
        Hq, Dh = 32, 128
        Hkv, Sk = A_k_cache.shape[1], A_k_cache.shape[2]
        W = min(4096, max(256, Sk // 4))
        F = B_w1.shape[1]
        kernel, scratch = make_kernel(B, D, Hq, Hkv, Sk, Dh, F, W, cfg)
        any_spec = pl.BlockSpec(memory_space=pl.ANY)
        out = pl.pallas_call(
            kernel,
            out_shape=jax.ShapeDtypeStruct((B, D), A_x.dtype),
            in_specs=[any_spec] * 9,
            out_specs=pl.BlockSpec(memory_space=pltpu.VMEM),
            scratch_shapes=scratch,
            compiler_params=pltpu.CompilerParams(
                vmem_limit_bytes=110 * 1024 * 1024,
                disable_semaphore_checks=True),
        )(A_x.reshape(B, D), A_k_cache, A_v_cache, A_wq, A_wo, B_w1,
          B_b1.reshape(F // LANE, LANE), B_w2, B_b2.reshape(D // LANE, LANE))
        return out.reshape(B, Sq, D)

    return fn


pallas_interleave_layers__sliding_block_cached__mixer_channel_mlp__decode_kernel = build({"nq":1, "nkv":1, "nsub":4, "tr_per":12, "ns":6, "gap":14})
```

```python
import math

import jax
import jax.numpy as jnp
import jax.experimental.pallas as pl
import jax.experimental.pallas.tpu as pltpu

F32 = jnp.float32
BF16 = jnp.bfloat16
U32 = jnp.uint32
EPS = 1e-5
LANE = 128
LOG2E = math.log2(math.e)

BLOCK_TILES = 16
PHASE = dict(k=5, v=5, wq=5, wo=5, w1=13)
N_STREAMS = 6
W2_STREAMS = 4
W2_SLICES = 2
LAG = (34, 62)
GAP = 14
TAIL_ROWS = 1536
TAIL_PIECE = 128
TAIL = ((0, 2, 6), (2, 2, 6), (4, 1, 6), (5, 1, 4), (6, 1, 0), (7, 1, 0))
PV_LAG = 4


def _stats(x):
    m = jnp.mean(x, axis=-1, keepdims=True)
    d = x - m
    v = jnp.mean(d * d, axis=-1, keepdims=True)
    return m, v, d


def _ln(x):
    _, v, d = _stats(x)
    return d * jax.lax.rsqrt(v + EPS)


def _hilo(x):
    hi = x.astype(BF16).astype(F32)
    return jnp.concatenate([hi, x - hi], axis=0).astype(BF16)


def _hilo_ones(x):
    hi = x.astype(BF16).astype(F32)
    row = jax.lax.broadcasted_iota(jnp.int32, x.shape, 0)
    ones = jnp.where(row == 0, 1.0, 0.0).astype(F32)
    return jnp.concatenate([hi, x - hi, ones, jnp.zeros_like(x)], axis=0).astype(BF16)


def _fold(y):
    n = y.shape[0] // 2
    return y[:n] + y[n:]


def _dot(a, b):
    return jnp.dot(a, b, preferred_element_type=F32)


def _dot_nt(a, b):
    return jax.lax.dot_general(a, b, (((1,), (1,)), ((), ())), preferred_element_type=F32)


def _unpack(p):
    return pltpu.bitcast(p, BF16)


def _splits(total, step):
    return [(r, min(step, total - r)) for r in range(0, total, step)]


def _tile_blocks(n_tiles, phase):
    cuts = [0] + [t for t in range(1, n_tiles) if (t - phase) % BLOCK_TILES == 0] + [n_tiles]
    return list(zip(cuts[:-1], cuts[1:]))


class _Unit:
    def __init__(self, whole, sem):
        self.whole = whole
        self.sem = sem
        self.ready = 0


def _make_kernel(B, D, Hq, Hkv, Sk, Dh, F, W):
    rep = Hq // Hkv
    G = B * Hkv
    HD = Hq * Dh
    T = TAIL_ROWS
    R = F - T
    NF = F // LANE
    ND = D // LANE
    RS = R // (2 * W2_STREAMS)
    SL = RS // W2_SLICES
    scale = Dh ** -0.5
    n_sems = 3 + 5 + W2_SLICES + len(TAIL)
    assert B == 8 and rep == 8 and Dh == LANE and SL % LANE == 0
    assert sum(nj for _, nj, _ in TAIL) == ND

    def kernel(x_hbm, k_hbm, v_hbm, wq_hbm, wo_hbm, w1_hbm, b1_hbm, w2_hbm, b2_hbm,
               o_ref,
               x_v, b1_v, b2_v,
               wq_s, k_s, v_s, wo_s, w1_s, w2_s, w2t,
               wq_p, kt_p, wo_p, w1_p, w2_p,
               q_scr, o_scr, s_scr,
               sems, fence):
        sem_iter = iter(range(n_sems))

        smalls = []
        for src, dst in ((x_hbm, x_v), (b1_hbm, b1_v), (b2_hbm, b2_v)):
            c = pltpu.make_async_copy(src, dst, sems.at[next(sem_iter)])
            c.start(priority=0)
            smalls.append(c)

        queues = ([], [])

        def new_unit(whole):
            return _Unit(whole, sems.at[next(sem_iter)])

        def add_region(blocks, u):
            n, k = len(blocks), 2 * N_STREAMS
            subs = [blocks[n * i // k:n * (i + 1) // k] for i in range(k)]
            for t in range(2):
                ss = subs[t * N_STREAMS:(t + 1) * N_STREAMS]
                for i in range(max(len(x) for x in ss)):
                    queues[t].extend((x[i], u) for x in ss if i < len(x))

        def weight_unit(hbm, stage, phase):
            u = new_unit(stage)
            nt = hbm.shape[1] // LANE
            blocks = []
            for a, b in _tile_blocks(hbm.shape[0] // 8 * nt, phase):
                blk = []
                while a < b:
                    g, j = divmod(a, nt)
                    if j == 0 and b - a >= nt:
                        ng = (b - a) // nt
                        idx = (pl.ds(g * 8, ng * 8),)
                        a += ng * nt
                    else:
                        e = min(b - g * nt, nt)
                        idx = (pl.ds(g * 8, 8), pl.ds(j * LANE, (e - j) * LANE))
                        a = g * nt + e
                    blk.append((hbm.at[idx], stage.at[idx]))
                blocks.append(blk)
            add_region(blocks, u)
            return u

        def cache_unit(hbm, stage, phase):
            u = new_unit(stage)
            add_region([[(hbm.at[b, kv, pl.ds(Sk - W + a * 8, (e - a) * 8), :],
                          stage.at[b, kv, pl.ds(a * 8, (e - a) * 8), :])]
                        for b in range(B) for kv in range(Hkv)
                        for a, e in _tile_blocks(W // 8, phase)], u)
            return u

        u_wq = weight_unit(wq_hbm, wq_s, PHASE["wq"])
        u_k = cache_unit(k_hbm, k_s, PHASE["k"])
        u_v = cache_unit(v_hbm, v_s, PHASE["v"])
        u_wo = weight_unit(wo_hbm, wo_s, PHASE["wo"])
        u_w1 = weight_unit(w1_hbm, w1_s, PHASE["w1"])
        u_w2 = []
        for i in range(W2_SLICES):
            u = new_unit(w2_s.at[:, pl.ds(i * SL, SL)])
            u_w2.append(u)
            for r, p in _splits(SL, BLOCK_TILES * 8 // ND):
                for s in range(2 * W2_STREAMS):
                    queues[s // W2_STREAMS].append(
                        ([(w2_hbm.at[pl.ds(s * RS + i * SL + r, p)],
                           w2_s.at[s, pl.ds(i * SL + r, p)])], u))
        u_t = []
        for j0, nj, n0 in TAIL:
            u = new_unit(w2t.at[pl.ds(j0, nj)])
            u_t.append(u)
            for i, (r, p) in enumerate(_splits(T, TAIL_PIECE)):
                for j in range(j0, j0 + nj):
                    queues[0 if i < n0 else 1].append(
                        ([(w2_hbm.at[pl.ds(R + r, p), pl.ds(j * LANE, LANE)],
                           w2t.at[j, pl.ds(r, p), :])], u))

        n_slots = len(queues[0])
        lead = len(queues[1]) - n_slots
        assert lead >= 0
        for i, (_, u) in enumerate(queues[0]):
            u.ready = max(u.ready, i + 1 + LAG[0])
        for i, (_, u) in enumerate(queues[1]):
            u.ready = max(u.ready, i + 1 - lead + LAG[1])
        cur = [-lead]

        def barrier():
            pl.semaphore_signal(fence, 1)
            pl.semaphore_wait(fence, 1)

        def issue_until(slot):
            while cur[0] < min(slot, n_slots):
                for t, i in ((0, cur[0]), (1, cur[0] + lead)):
                    if i >= 0:
                        blk, u = queues[t][i]
                        for src, dst in blk:
                            pltpu.make_async_copy(src, dst, u.sem).start(priority=t)
                cur[0] += 1

        def need(u):
            if cur[0] < min(u.ready, n_slots):
                barrier()
                issue_until(u.ready)
            pltpu.make_async_copy(u.whole, u.whole, u.sem).wait()

        def gap():
            if cur[0] < n_slots:
                barrier()
                issue_until(cur[0] + GAP)
                barrier()

        def mm_retile(lhs, stage, packed):
            acc = None
            for r, p in _splits(stage.shape[0], stage.shape[0] // 4):
                if r:
                    gap()
                w = stage[pl.ds(r, p), :]
                packed[pl.ds(r // 2, p // 2), :] = pltpu.bitcast(w, U32)
                part = _dot(lhs[:, r:r + p], w)
                acc = part if acc is None else part + acc
            return acc

        def scatter_q(q):
            for h in range(Hq):
                q_scr[pl.ds(h * B, B), :] = q[:, h * Dh:(h + 1) * Dh]

        def group_rows(b, kv):
            return pl.ds(kv * rep * B + b, rep, stride=B)

        def softmax_pv(s, b, kv, c):
            m = jnp.max(s, axis=-1, keepdims=True)
            p = jnp.exp2((s - m) * c)
            l = jnp.sum(p, axis=-1, keepdims=True)
            o_scr[group_rows(b, kv), :] = _fold(_dot(_hilo(p), v_s[b, kv])) / l

        def gather_o():
            return _hilo(jnp.concatenate([o_scr[pl.ds(h * B, B), :] for h in range(Hq)], axis=1))

        def bias_row(b_v):
            bf = b_v[...].astype(F32)
            return jnp.concatenate([bf[j:j + 1, :] for j in range(bf.shape[0])], axis=1)

        todo_t = [(b, kv) for b in range(B) for kv in range(Hkv)]

        def transpose_k(count):
            for n in range(min(count, len(todo_t))):
                if n % 3 == 0:
                    gap()
                b, kv = todo_t.pop(0)
                kt_p[b * Hkv + kv] = pltpu.bitcast(k_s[b, kv].T, U32)

        issue_until(8)
        for c in smalls:
            c.wait()
        x0 = x_v[...].astype(F32)
        b1 = bias_row(b1_v)
        b2 = bias_row(b2_v)
        lhs = _hilo_ones(_ln(x0))

        need(u_wq)
        q = mm_retile(lhs, wq_s, wq_p)
        cs_q = q[2 * B:2 * B + 1, :]
        scatter_q(_fold(q[:2 * B]))

        need(u_k)
        for b in range(B):
            if b and b % 2 == 0:
                gap()
            for kv in range(Hkv):
                s_scr[b * Hkv + kv] = _fold(_dot_nt(_hilo(q_scr[group_rows(b, kv), :]), k_s[b, kv]))
        transpose_k(12)

        need(u_v)
        for b in range(B):
            if b and b % 4 == 0:
                gap()
            for kv in range(Hkv):
                softmax_pv(s_scr[b * Hkv + kv], b, kv, scale * LOG2E)
        transpose_k(12)
        o = gather_o()

        need(u_wo)
        att = mm_retile(o, wo_s, wo_p)
        transpose_k(G)
        x1 = x0 + _fold(att)
        lhs = _hilo_ones(_ln(_ln(x1)))

        need(u_w1)
        pre = mm_retile(lhs, w1_s, w1_p)
        cs_1 = pre[2 * B:2 * B + 1, :]
        h = _hilo(jax.nn.gelu(_fold(pre[:2 * B]) + b1, approximate=True))

        x2m = x1 + b2
        for i, u in enumerate(u_w2):
            need(u)
            w = w2_s[:, pl.ds(i * SL, SL), :]
            w2_p[:, pl.ds(i * SL // 2, SL // 2), :] = pltpu.bitcast(w, U32)
            hs = jnp.concatenate([h[:, s * RS + i * SL:s * RS + (i + 1) * SL]
                                  for s in range(2 * W2_STREAMS)], axis=1)
            x2m = x2m + _fold(_dot(hs, w.reshape(2 * W2_STREAMS * SL, D)))

        ht = h[:, R:]
        x2_parts = []
        q_raw = None
        for (j0, nj, _), u in zip(TAIL, u_t):
            need(u)
            x2c = jnp.concatenate([x2m[:, j * LANE:(j + 1) * LANE] + _fold(_dot(ht, w2t[j]))
                                   for j in range(j0, j0 + nj)], axis=1)
            x2_parts.append(x2c)
            part = _fold(_dot(_hilo(x2c), _unpack(wq_p[pl.ds(j0 * LANE // 2, nj * LANE // 2), :])))
            q_raw = part if q_raw is None else q_raw + part
        x2 = jnp.concatenate(x2_parts, axis=1)

        m, v, _ = _stats(x2)
        c_exp = jax.lax.rsqrt(v + EPS) * (scale * LOG2E)
        scatter_q(q_raw - m * cs_q)
        order = [(b, kv) for kv in range(Hkv) for b in range(B)]
        scores = {}
        for i in range(G + PV_LAG):
            if i < G:
                b, kv = order[i]
                scores[i] = _fold(_dot(_hilo(q_scr[group_rows(b, kv), :]), _unpack(kt_p[b * Hkv + kv])))
            if i >= PV_LAG:
                b, kv = order[i - PV_LAG]
                softmax_pv(scores.pop(i - PV_LAG), b, kv, c_exp[b:b + 1, :])
        x3 = x2 + _fold(_dot(gather_o(), _unpack(wo_p[...])))

        pr = _fold(_dot(_hilo(x3), _unpack(w1_p[...])))
        m1, v1, d1 = _stats(x3)
        rs1 = jax.lax.rsqrt(v1 + EPS)
        m2, v2, _ = _stats(d1 * rs1)
        rs2 = jax.lax.rsqrt(v2 + EPS)
        a = rs1 * rs2
        pre = pr * a - (m1 * a + m2 * rs2) * cs_1 + b1
        h = _hilo(jax.nn.gelu(pre, approximate=True))
        y = _dot(h[:, :R], _unpack(w2_p[...].reshape(R // 2, D)))
        ht = h[:, R:]
        yt = jnp.concatenate([_dot(ht, w2t[j]) for j in range(ND)], axis=1)
        o_ref[...] = ((x3 + b2 + _fold(y)) + _fold(yt)).astype(o_ref.dtype)

    scratch = [
        pltpu.VMEM((B, D), BF16), pltpu.VMEM((NF, LANE), BF16), pltpu.VMEM((ND, LANE), BF16),
        pltpu.VMEM((D, HD), BF16), pltpu.VMEM((B, Hkv, W, Dh), BF16), pltpu.VMEM((B, Hkv, W, Dh), BF16),
        pltpu.VMEM((HD, D), BF16), pltpu.VMEM((D, F), BF16), pltpu.VMEM((2 * W2_STREAMS, RS, D), BF16),
        pltpu.VMEM((ND, T, LANE), BF16),
        pltpu.VMEM((D // 2, HD), U32), pltpu.VMEM((G, Dh // 2, W), U32), pltpu.VMEM((HD // 2, D), U32),
        pltpu.VMEM((D // 2, F), U32), pltpu.VMEM((2 * W2_STREAMS, RS // 2, D), U32),
        pltpu.VMEM((Hq * B, Dh), F32), pltpu.VMEM((Hq * B, Dh), F32), pltpu.VMEM((G, rep, W), F32),
        pltpu.SemaphoreType.DMA((n_sems,)), pltpu.SemaphoreType.REGULAR,
    ]
    return kernel, scratch


@jax.jit
def pallas_interleave_layers__sliding_block_cached__mixer_channel_mlp__decode_kernel(
    A_x: jax.Array,
    A_k_cache: jax.Array,
    A_v_cache: jax.Array,
    A_wq: jax.Array,
    A_wo: jax.Array,
    B_x: jax.Array,
    B_w1: jax.Array,
    B_b1: jax.Array,
    B_w2: jax.Array,
    B_b2: jax.Array,
):
    del B_x
    B, Sq, D = A_x.shape
    assert Sq == 1
    Hq, Dh = 32, 128
    Hkv, Sk = A_k_cache.shape[1], A_k_cache.shape[2]
    W = min(4096, max(256, Sk // 4))
    F = B_w1.shape[1]
    kernel, scratch = _make_kernel(B, D, Hq, Hkv, Sk, Dh, F, W)
    out = pl.pallas_call(
        kernel,
        out_shape=jax.ShapeDtypeStruct((B, D), A_x.dtype),
        in_specs=[pl.BlockSpec(memory_space=pl.ANY)] * 9,
        out_specs=pl.BlockSpec(memory_space=pltpu.VMEM),
        scratch_shapes=scratch,
        compiler_params=pltpu.CompilerParams(
            vmem_limit_bytes=110 * 1024 * 1024,
            disable_semaphore_checks=True),
    )(A_x.reshape(B, D), A_k_cache, A_v_cache, A_wq, A_wo, B_w1,
      B_b1.reshape(F // LANE, LANE), B_w2, B_b2.reshape(D // LANE, LANE))
    return out.reshape(B, Sq, D)
```

```python
import math

import jax
import jax.numpy as jnp
import jax.experimental.pallas as pl
import jax.experimental.pallas.tpu as pltpu

F32 = jnp.float32
BF16 = jnp.bfloat16
U32 = jnp.uint32
EPS = 1e-5
LANE = 128
LOG2E = math.log2(math.e)

BLOCK_TILES = 16
PHASE = dict(k=5, v=5, wq=5, wo=5, w1=13)
N_STREAMS = 6
W2_STREAMS = 4
W2_SLICES = 2
LAG = (34, 62)
GAP = 14
TAIL_ROWS = 1536
TAIL_PIECE = 128
TAIL = ((0, 2, 6), (2, 2, 6), (4, 1, 6), (5, 1, 4), (6, 1, 0), (7, 1, 0))
PV_LAG = 4


def _stats(x):
    m = jnp.mean(x, axis=-1, keepdims=True)
    d = x - m
    v = jnp.mean(d * d, axis=-1, keepdims=True)
    return m, v, d


def _ln(x):
    _, v, d = _stats(x)
    return d * jax.lax.rsqrt(v + EPS)


def _hilo(x):
    hi = x.astype(BF16).astype(F32)
    return jnp.concatenate([hi, x - hi], axis=0).astype(BF16)


def _hilo_ones(x):
    hi = x.astype(BF16).astype(F32)
    row = jax.lax.broadcasted_iota(jnp.int32, x.shape, 0)
    ones = jnp.where(row == 0, 1.0, 0.0).astype(F32)
    return jnp.concatenate([hi, x - hi, ones, jnp.zeros_like(x)], axis=0).astype(BF16)


def _fold(y):
    n = y.shape[0] // 2
    return y[:n] + y[n:]


def _dot(a, b):
    return jnp.dot(a, b, preferred_element_type=F32)


def _dot_nt(a, b):
    return jax.lax.dot_general(a, b, (((1,), (1,)), ((), ())), preferred_element_type=F32)


def _unpack(p):
    return pltpu.bitcast(p, BF16)


def _splits(total, step):
    return [(r, min(step, total - r)) for r in range(0, total, step)]


def _tile_blocks(n_tiles, phase):
    cuts = [0] + [t for t in range(1, n_tiles) if (t - phase) % BLOCK_TILES == 0] + [n_tiles]
    return list(zip(cuts[:-1], cuts[1:]))


class _Unit:
    def __init__(self, whole, sem):
        self.whole = whole
        self.sem = sem
        self.ready = 0


def _make_kernel(B, D, Hq, Hkv, Sk, Dh, F, W):
    rep = Hq // Hkv
    G = B * Hkv
    HD = Hq * Dh
    T = TAIL_ROWS
    R = F - T
    NF = F // LANE
    ND = D // LANE
    RS = R // (2 * W2_STREAMS)
    SL = RS // W2_SLICES
    scale = Dh ** -0.5
    n_sems = 3 + 5 + W2_SLICES + len(TAIL)
    assert B == 8 and rep == 8 and Dh == LANE and SL % LANE == 0
    assert sum(nj for _, nj, _ in TAIL) == ND

    def kernel(x_hbm, k_hbm, v_hbm, wq_hbm, wo_hbm, w1_hbm, b1_hbm, w2_hbm, b2_hbm,
               o_ref,
               x_v, b1_v, b2_v,
               wq_s, k_s, v_s, wo_s, w1_s, w2_s, w2t,
               wq_p, kt_p, wo_p, w1_p, w2_p,
               q_scr, o_scr, s_scr,
               sems, fence):
        sem_iter = iter(range(n_sems))

        smalls = []
        for src, dst in ((x_hbm, x_v), (b1_hbm, b1_v), (b2_hbm, b2_v)):
            c = pltpu.make_async_copy(src, dst, sems.at[next(sem_iter)])
            c.start(priority=0)
            smalls.append(c)

        queues = ([], [])

        def new_unit(whole):
            return _Unit(whole, sems.at[next(sem_iter)])

        def add_region(blocks, u):
            n, k = len(blocks), 2 * N_STREAMS
            subs = [blocks[n * i // k:n * (i + 1) // k] for i in range(k)]
            for t in range(2):
                ss = subs[t * N_STREAMS:(t + 1) * N_STREAMS]
                for i in range(max(len(x) for x in ss)):
                    queues[t].extend((x[i], u) for x in ss if i < len(x))

        def weight_unit(hbm, stage, phase):
            u = new_unit(stage)
            nt = hbm.shape[1] // LANE
            blocks = []
            for a, b in _tile_blocks(hbm.shape[0] // 8 * nt, phase):
                blk = []
                while a < b:
                    g, j = divmod(a, nt)
                    if j == 0 and b - a >= nt:
                        ng = (b - a) // nt
                        idx = (pl.ds(g * 8, ng * 8),)
                        a += ng * nt
                    else:
                        e = min(b - g * nt, nt)
                        idx = (pl.ds(g * 8, 8), pl.ds(j * LANE, (e - j) * LANE))
                        a = g * nt + e
                    blk.append((hbm.at[idx], stage.at[idx]))
                blocks.append(blk)
            add_region(blocks, u)
            return u

        def cache_unit(hbm, stage, phase):
            u = new_unit(stage)
            add_region([[(hbm.at[b, kv, pl.ds(Sk - W + a * 8, (e - a) * 8), :],
                          stage.at[b, kv, pl.ds(a * 8, (e - a) * 8), :])]
                        for b in range(B) for kv in range(Hkv)
                        for a, e in _tile_blocks(W // 8, phase)], u)
            return u

        u_wq = weight_unit(wq_hbm, wq_s, PHASE["wq"])
        u_k = cache_unit(k_hbm, k_s, PHASE["k"])
        u_v = cache_unit(v_hbm, v_s, PHASE["v"])
        u_wo = weight_unit(wo_hbm, wo_s, PHASE["wo"])
        u_w1 = weight_unit(w1_hbm, w1_s, PHASE["w1"])
        u_w2 = []
        for i in range(W2_SLICES):
            u = new_unit(w2_s.at[:, pl.ds(i * SL, SL)])
            u_w2.append(u)
            for r, p in _splits(SL, BLOCK_TILES * 8 // ND):
                for s in range(2 * W2_STREAMS):
                    queues[s // W2_STREAMS].append(
                        ([(w2_hbm.at[pl.ds(s * RS + i * SL + r, p)],
                           w2_s.at[s, pl.ds(i * SL + r, p)])], u))
        u_t = []
        for j0, nj, n0 in TAIL:
            u = new_unit(w2t.at[pl.ds(j0, nj)])
            u_t.append(u)
            for i, (r, p) in enumerate(_splits(T, TAIL_PIECE)):
                for j in range(j0, j0 + nj):
                    queues[0 if i < n0 else 1].append(
                        ([(w2_hbm.at[pl.ds(R + r, p), pl.ds(j * LANE, LANE)],
                           w2t.at[j, pl.ds(r, p), :])], u))

        n_slots = len(queues[0])
        lead = len(queues[1]) - n_slots
        assert lead >= 0
        for i, (_, u) in enumerate(queues[0]):
            u.ready = max(u.ready, i + 1 + LAG[0])
        for i, (_, u) in enumerate(queues[1]):
            u.ready = max(u.ready, i + 1 - lead + LAG[1])
        cur = [-lead]

        def barrier():
            pl.semaphore_signal(fence, 1)
            pl.semaphore_wait(fence, 1)

        def issue_until(slot):
            while cur[0] < min(slot, n_slots):
                for t, i in ((0, cur[0]), (1, cur[0] + lead)):
                    if i >= 0:
                        blk, u = queues[t][i]
                        for src, dst in blk:
                            pltpu.make_async_copy(src, dst, u.sem).start(priority=t)
                cur[0] += 1

        def need(u):
            if cur[0] < min(u.ready, n_slots):
                barrier()
                issue_until(u.ready)
            pltpu.make_async_copy(u.whole, u.whole, u.sem).wait()

        def gap():
            if cur[0] < n_slots:
                barrier()
                issue_until(cur[0] + GAP)
                barrier()

        def mm_retile(lhs, stage, packed):
            acc = None
            for r, p in _splits(stage.shape[0], stage.shape[0] // 4):
                if r:
                    gap()
                w = stage[pl.ds(r, p), :]
                packed[pl.ds(r // 2, p // 2), :] = pltpu.bitcast(w, U32)
                part = _dot(lhs[:, r:r + p], w)
                acc = part if acc is None else part + acc
            return acc

        def scatter_q(q):
            for h in range(Hq):
                q_scr[pl.ds(h * B, B), :] = q[:, h * Dh:(h + 1) * Dh]

        def group_rows(b, kv):
            return pl.ds(kv * rep * B + b, rep, stride=B)

        def softmax_pv(s, b, kv, c):
            m = jnp.max(s, axis=-1, keepdims=True)
            p = jnp.exp2((s - m) * c)
            l = jnp.sum(p, axis=-1, keepdims=True)
            o_scr[group_rows(b, kv), :] = _fold(_dot(_hilo(p), v_s[b, kv])) / l

        def gather_o():
            return _hilo(jnp.concatenate([o_scr[pl.ds(h * B, B), :] for h in range(Hq)], axis=1))

        def bias_row(b_v):
            bf = b_v[...].astype(F32)
            return jnp.concatenate([bf[j:j + 1, :] for j in range(bf.shape[0])], axis=1)

        todo_t = [(b, kv) for b in range(B) for kv in range(Hkv)]

        def transpose_k(count):
            for n in range(min(count, len(todo_t))):
                if n % 3 == 0:
                    gap()
                b, kv = todo_t.pop(0)
                kt_p[b * Hkv + kv] = pltpu.bitcast(k_s[b, kv].T, U32)

        issue_until(8)
        for c in smalls:
            c.wait()
        x0 = x_v[...].astype(F32)
        b1 = bias_row(b1_v)
        b2 = bias_row(b2_v)
        lhs = _hilo_ones(_ln(x0))

        need(u_wq)
        q = mm_retile(lhs, wq_s, wq_p)
        cs_q = q[2 * B:2 * B + 1, :]
        scatter_q(_fold(q[:2 * B]))

        need(u_k)
        for b in range(B):
            if b and b % 2 == 0:
                gap()
            for kv in range(Hkv):
                s_scr[b * Hkv + kv] = _fold(_dot_nt(_hilo(q_scr[group_rows(b, kv), :]), k_s[b, kv]))
        transpose_k(12)

        need(u_v)
        for b in range(B):
            if b and b % 4 == 0:
                gap()
            for kv in range(Hkv):
                softmax_pv(s_scr[b * Hkv + kv], b, kv, scale * LOG2E)
        transpose_k(12)
        o = gather_o()

        need(u_wo)
        att = mm_retile(o, wo_s, wo_p)
        transpose_k(G)
        x1 = x0 + _fold(att)
        lhs = _hilo_ones(_ln(_ln(x1)))

        need(u_w1)
        pre = mm_retile(lhs, w1_s, w1_p)
        cs_1 = pre[2 * B:2 * B + 1, :]
        h = _hilo(jax.nn.gelu(_fold(pre[:2 * B]) + b1, approximate=True))

        x2m = x1 + b2
        for i, u in enumerate(u_w2):
            need(u)
            w = w2_s[:, pl.ds(i * SL, SL), :]
            w2_p[:, pl.ds(i * SL // 2, SL // 2), :] = pltpu.bitcast(w, U32)
            hs = jnp.concatenate([h[:, s * RS + i * SL:s * RS + (i + 1) * SL]
                                  for s in range(2 * W2_STREAMS)], axis=1)
            x2m = x2m + _fold(_dot(hs, w.reshape(2 * W2_STREAMS * SL, D)))

        ht = h[:, R:]
        x2_parts = []
        q_raw = None
        for (j0, nj, _), u in zip(TAIL, u_t):
            need(u)
            x2c = jnp.concatenate([x2m[:, j * LANE:(j + 1) * LANE] + _fold(_dot(ht, w2t[j]))
                                   for j in range(j0, j0 + nj)], axis=1)
            x2_parts.append(x2c)
            part = _fold(_dot(_hilo(x2c), _unpack(wq_p[pl.ds(j0 * LANE // 2, nj * LANE // 2), :])))
            q_raw = part if q_raw is None else q_raw + part
        x2 = jnp.concatenate(x2_parts, axis=1)
        assert cur[0] == n_slots and not todo_t

        m, v, _ = _stats(x2)
        c_exp = jax.lax.rsqrt(v + EPS) * (scale * LOG2E)
        scatter_q(q_raw - m * cs_q)
        order = [(b, kv) for kv in range(Hkv) for b in range(B)]
        scores = {}
        for i in range(G + PV_LAG):
            if i < G:
                b, kv = order[i]
                scores[i] = _fold(_dot(_hilo(q_scr[group_rows(b, kv), :]), _unpack(kt_p[b * Hkv + kv])))
            if i >= PV_LAG:
                b, kv = order[i - PV_LAG]
                softmax_pv(scores.pop(i - PV_LAG), b, kv, c_exp[b:b + 1, :])
        x3 = x2 + _fold(_dot(gather_o(), _unpack(wo_p[...])))

        x3h = _hilo(x3)
        kc, n1 = D // 2, 4 * LANE
        pr = jnp.concatenate([
            _fold(_dot(x3h[:, :kc], _unpack(w1_p[pl.ds(0, kc // 2), pl.ds(0, n1)])))
            + _fold(_dot(x3h[:, kc:], _unpack(w1_p[pl.ds(kc // 2, kc // 2), pl.ds(0, n1)]))),
            _fold(_dot(x3h, _unpack(w1_p[:, pl.ds(n1, F - n1)])))], axis=1)
        m1, v1, d1 = _stats(x3)
        rs1 = jax.lax.rsqrt(v1 + EPS)
        m2, v2, _ = _stats(d1 * rs1)
        rs2 = jax.lax.rsqrt(v2 + EPS)
        a = rs1 * rs2
        pre = pr * a - (m1 * a + m2 * rs2) * cs_1 + b1
        h = _hilo(jax.nn.gelu(pre, approximate=True))
        y = _dot(h[:, :R], _unpack(w2_p[...].reshape(R // 2, D)))
        ht = h[:, R:]
        yt = jnp.concatenate([_dot(ht, w2t[j]) for j in range(ND)], axis=1)
        o_ref[...] = ((x3 + b2 + _fold(y)) + _fold(yt)).astype(o_ref.dtype)

    scratch = [
        pltpu.VMEM((B, D), BF16), pltpu.VMEM((NF, LANE), BF16), pltpu.VMEM((ND, LANE), BF16),
        pltpu.VMEM((D, HD), BF16), pltpu.VMEM((B, Hkv, W, Dh), BF16), pltpu.VMEM((B, Hkv, W, Dh), BF16),
        pltpu.VMEM((HD, D), BF16), pltpu.VMEM((D, F), BF16), pltpu.VMEM((2 * W2_STREAMS, RS, D), BF16),
        pltpu.VMEM((ND, T, LANE), BF16),
        pltpu.VMEM((D // 2, HD), U32), pltpu.VMEM((G, Dh // 2, W), U32), pltpu.VMEM((HD // 2, D), U32),
        pltpu.VMEM((D // 2, F), U32), pltpu.VMEM((2 * W2_STREAMS, RS // 2, D), U32),
        pltpu.VMEM((Hq * B, Dh), F32), pltpu.VMEM((Hq * B, Dh), F32), pltpu.VMEM((G, rep, W), F32),
        pltpu.SemaphoreType.DMA((n_sems,)), pltpu.SemaphoreType.REGULAR,
    ]
    return kernel, scratch


@jax.jit
def pallas_interleave_layers__sliding_block_cached__mixer_channel_mlp__decode_kernel(
    A_x: jax.Array,
    A_k_cache: jax.Array,
    A_v_cache: jax.Array,
    A_wq: jax.Array,
    A_wo: jax.Array,
    B_x: jax.Array,
    B_w1: jax.Array,
    B_b1: jax.Array,
    B_w2: jax.Array,
    B_b2: jax.Array,
):
    del B_x
    B, Sq, D = A_x.shape
    assert Sq == 1
    Hq, Dh = 32, 128
    Hkv, Sk = A_k_cache.shape[1], A_k_cache.shape[2]
    W = min(4096, max(256, Sk // 4))
    F = B_w1.shape[1]
    kernel, scratch = _make_kernel(B, D, Hq, Hkv, Sk, Dh, F, W)
    out = pl.pallas_call(
        kernel,
        out_shape=jax.ShapeDtypeStruct((B, D), A_x.dtype),
        in_specs=[pl.BlockSpec(memory_space=pl.ANY)] * 9,
        out_specs=pl.BlockSpec(memory_space=pltpu.VMEM),
        scratch_shapes=scratch,
        compiler_params=pltpu.CompilerParams(
            vmem_limit_bytes=110 * 1024 * 1024,
            disable_semaphore_checks=True),
    )(A_x.reshape(B, D), A_k_cache, A_v_cache, A_wq, A_wo, B_w1,
      B_b1.reshape(F // LANE, LANE), B_w2, B_b2.reshape(D // LANE, LANE))
    return out.reshape(B, Sq, D)
```
